```python
import jax
import jax.numpy as jnp

def _softmax(x, axis=-1):
    return jax.nn.softmax(x, axis=axis)

def _gelu(x):
    return jax.nn.gelu(x, approximate=True)

def _silu(x):
    return jax.nn.silu(x)

def _sigmoid(x):
    return jax.nn.sigmoid(x)

def _layernorm(x, axis=-1, eps=1e-05):
    m = jnp.mean(x, axis=axis, keepdims=True)
    v = jnp.var(x, axis=axis, keepdims=True)
    return (x - m) / jnp.sqrt(v + eps)

def _scatter_add(tgt, idx, src, axis=0):
    return tgt.at[idx].add(src)

def _segment_sum(src, seg, n):
    return jax.ops.segment_sum(src, seg, n)

class _Rng:

    def __init__(self, key):
        self._k = key

    def _next(self):
        self._k, sub = jax.random.split(self._k)
        return sub

    def normal(self, shape):
        return jax.random.normal(self._next(), shape, dtype=jnp.bfloat16)

    def randint(self, lo, hi, shape):
        return jax.random.randint(self._next(), shape, lo, hi, dtype=jnp.int32)

    def uniform(self, shape, lo=0.0, hi=1.0):
        return jax.random.uniform(self._next(), shape, jnp.bfloat16, lo, hi)

    def permutation(self, n):
        return jax.random.permutation(self._next(), n)
kernel_name = 'adaLN_cond__sliding_block_cached__mixer_s_mlp__decode'

def setup_inputs():
    _rng = _Rng(jax.random.key(int.from_bytes(__import__("os").urandom(4), "little")))
    _w = lambda a: (lambda t: t.astype(jnp.bfloat16) if jnp.issubdtype(t.dtype, jnp.floating) else t)(jnp.asarray(a))

    def _A_setup():
        B, Sq, D = (1, 1, 448)
        Hq, Hkv, Sk, Dh = (16, 8, 65536, 256)
        assert Hq % Hkv == 0, (Hq, Hkv)
        return {'x': _w((lambda *s: _rng.normal(s) * 0.05)(B, Sq, D)), 'k_cache': _w((lambda *s: _rng.normal(s) * 0.05)(B, Hkv, Sk, Dh)), 'v_cache': _w((lambda *s: _rng.normal(s) * 0.05)(B, Hkv, Sk, Dh)), 'wq': _w((lambda *s: _rng.normal(s) * 0.05)(D, Hq * Dh) * D ** (-0.5)), 'wo': _w((lambda *s: _rng.normal(s) * 0.05)(Hq * Dh, D) * (Hq * Dh) ** (-0.5))}
    _A_in = _A_setup()

    def _B_setup():
        B, S, D, F = (1, 1, 448, 1792)
        return {'x': _w((lambda *s: _rng.normal(s) * 0.05)(B, S, D)), 'w1': _w((lambda *s: _rng.normal(s) * 0.05)(D, D) * D ** (-0.5)), 'w2': _w((lambda *s: _rng.normal(s) * 0.05)(D, D) * D ** (-0.5)), 'w3': _w((lambda *s: _rng.normal(s) * 0.05)(D, F) * D ** (-0.5)), 'w4': _w((lambda *s: _rng.normal(s) * 0.05)(F, D) * F ** (-0.5))}
    _B_in = _B_setup()
    return {'A_x': _A_in['x'], 'A_k_cache': _A_in['k_cache'], 'A_v_cache': _A_in['v_cache'], 'A_wq': _A_in['wq'], 'A_wo': _A_in['wo'], 'B_x': _B_in['x'], 'B_w1': _B_in['w1'], 'B_w2': _B_in['w2'], 'B_w3': _B_in['w3'], 'B_w4': _B_in['w4'], 'c': _w((lambda *s: _rng.normal(s) * 0.05)(1, 448)), 'w_mod': _w((lambda *s: _rng.normal(s) * 0.05)(448, 6 * 448) * 448 ** (-0.5))}

def reference(A_x, A_k_cache, A_v_cache, A_wq, A_wo, B_x, B_w1, B_w2, B_w3, B_w4, c, w_mod):

    def _A_ref(x, k_cache, v_cache, wq, wo):
        B, Sq, D = x.shape
        Hq, Dh = (16, 256)
        Hkv, Sk = (k_cache.shape[1], k_cache.shape[2])
        W = min(4096, max(256, Sk // 4))
        rep = Hq // Hkv
        q = (lambda x, *d: x.transpose(*d))((x @ wq).reshape(B, Sq, Hq, Dh), 0, 2, 1, 3)
        k = jnp.repeat(k_cache[:, :, Sk - W:, :], rep, axis=1)
        v = jnp.repeat(v_cache[:, :, Sk - W:, :], rep, axis=1)
        scores = jnp.einsum('bhqd,bhkd->bhqk', q, k) * Dh ** (-0.5)
        p = _softmax(scores, axis=-1)
        o = jnp.einsum('bhqk,bhkd->bhqd', p, v)
        return (lambda x, *d: x.transpose(*d))(o, 0, 2, 1, 3).reshape(B, Sq, Hq * Dh) @ wo

    def _B_ref(x, w1, w2, w3, w4):
        B, S, D = x.shape
        h = _gelu(_layernorm(x, axis=-1) @ w1)
        c = D // 4
        g0 = jnp.pad(h[:, :, 0 * c:1 * c], ((0, 0), (1, 0), (0, 0)))[:, :S, :]
        g1 = jnp.pad(h[:, :, 1 * c:2 * c], ((0, 0), (0, 1), (0, 0)))[:, 1:, :]
        g2 = jnp.pad(h[:, :, 2 * c:3 * c], ((0, 0), (2, 0), (0, 0)))[:, :S, :]
        g3 = jnp.pad(h[:, :, 3 * c:], ((0, 0), (0, 2), (0, 0)))[:, 2:, :]
        hs = jnp.concatenate([g0, g1, g2, g3], axis=-1) @ w2
        x1 = x + hs
        h2 = _gelu(_layernorm(x1, axis=-1) @ w3) @ w4
        return x1 + h2
    x = A_x
    mod = (_silu(c) @ w_mod).reshape(c.shape[0], 6, 1, -1)
    sa, ca, ga, sb, cb, gb = (mod[:, 0].copy(), mod[:, 1].copy(), mod[:, 2].copy(), mod[:, 3].copy(), mod[:, 4].copy(), mod[:, 5].copy())
    h = _layernorm(x, axis=-1) * (1 + ca) + sa
    x = x + ga * _A_ref(h, A_k_cache, A_v_cache, A_wq, A_wo)
    h = _layernorm(x, axis=-1) * (1 + cb) + sb
    x = x + gb * _B_ref(h, B_w1, B_w2, B_w3, B_w4)
    return x
```

```python
import jax
import jax.numpy as jnp
from jax import lax
from jax.experimental import pallas as pl
from jax.experimental.pallas import tpu as pltpu

D, F = 448, 1792
HQ, HKV, DH = 16, 8, 256
WINDOW = 4096
EPS = 1e-5
ROWS = 8
LANES = 128
BLOCK, STEP = 1024, 16
LATE = 18 * LANES
W4_STAGES = ((0, 4), (4, 6), (6, 7))
GATE_STAGES = ((0, 80), (80, 104), (104, 112))
HEAD_START = 26
IN_FLIGHT = 32
BF16, F32 = jnp.bfloat16, jnp.float32

S_X, S_C, S_WM, S_WQ, S_WO, S_W3, S_K, S_V, S_W4, S_GATE, S_END = 0, 1, 2, 3, 4, 5, 6, 14, 22, 25, 28


def _layernorm(x):
    d = x - jnp.sum(x, axis=-1, keepdims=True) * (1.0 / D)
    return d * lax.rsqrt(jnp.sum(d * d, axis=-1, keepdims=True) * (1.0 / D) + EPS)


def _flat(blocks):
    return blocks.reshape(-1, blocks.shape[-1])


def _dot(a, blocks):
    return lax.dot_general(a, _flat(blocks), (((1,), (0,)), ((), ())), preferred_element_type=F32)


def _dot_t(a, blocks):
    return lax.dot_general(a, _flat(blocks), (((1,), (1,)), ((), ())), preferred_element_type=F32)


def _mix(*lists):
    return [item for group in zip(*lists, strict=True) for item in group]


def _tree(op, terms):
    while len(terms) > 1:
        terms = [op(a, b) for a, b in zip(terms[::2], terms[1::2])] + terms[len(terms) // 2 * 2:]
    return terms[0]


def _lane_tiles(x):
    return [x[:, t:t + LANES] for t in range(0, x.shape[1], LANES)]


def _kernel(x_hbm, c_hbm, wm_hbm, wq_hbm, k_hbm, v_hbm, wo_hbm, w3_hbm, w4_hbm, out_hbm,
            x_ref, c_ref, wm_ref, wq_ref, k_ref, v_ref, wo_ref, w3_ref, w4_ref,
            q_ref, s_ref, max_ref, attn_ref, mod_ref, cond_ref, out_ref, sems):
    def cache(hbm, ref, sem, h):
        n = WINDOW // BLOCK
        blocks = pl.ds((h + 1) * hbm.shape[0] // HKV - n, n)
        rows = [pl.ds((r + BLOCK // 4 * (h >> 1 & 1)) % BLOCK, STEP) for r in range(0, BLOCK, STEP)]
        return [pltpu.make_async_copy(hbm.at[blocks, r], ref.at[h, :, r], sems.at[sem + h]) for r in rows]

    def weight(hbm, ref, sem, first, n, tiles, col=0, rows=None):
        ends = [col + LANES * sum(tiles[:i]) for i in range(len(tiles) + 1)]
        pieces = [(pl.ds(first, n), pl.ds(r, 8), pl.ds(a, b - a))
                  for r in range(*(rows or (0, ref.shape[1])), 8) for a, b in zip(ends, ends[1:])]
        return [pltpu.make_async_copy(hbm.at[at], ref.at[at], sems.at[sem]) for at in pieces]

    keys = [cache(k_hbm, k_ref, S_K, h) for h in range(HKV)]
    values = [cache(v_hbm, v_ref, S_V, h) for h in range(HKV)]
    wide = _mix(*[weight(hbm, ref, sem, first, n, (4,) * 8)
                  for hbm, ref, sem in ((wq_hbm, wq_ref, S_WQ), (wo_hbm, wo_ref, S_WO))
                  for first, n in ((0, 4), (4, 3))])
    wm = weight(wm_hbm, wm_ref, S_WM, 0, 4, (4, 4, 4, 3, 3))
    w3 = weight(w3_hbm, w3_ref, S_W3, 0, 2, (7, 7))
    w4a, w4b = [weight(w4_hbm, w4_ref, S_W4, first, 2, (7, 7)) for first in (0, 2)]
    w4c, w4d, w4e = [weight(w4_hbm, w4_ref, S_W4 + stage, first, 1, (14,)) for stage, first in ((1, 4), (1, 5), (2, 6))]
    gate = [copy for i, rows in enumerate(GATE_STAGES)
            for copy in _mix(*[weight(wm_hbm, wm_ref, S_GATE + i, first, 2, (3,), LATE, rows) for first in (0, 2)])]

    def pair(heads, h):
        return _mix(heads[h], heads[h + 2])

    def ending(w3_part, w4_part):
        return w3_part[:-12] + _mix(w3_part[-12:], w4_part[:12]) + w4_part[12:]

    last = pair(values, 4)
    first = (pair(keys, 1) + pair(keys, 0) + pair(keys, 4) + pair(values, 0) + last[:-16]
             + ending(w3[:28], w4a + w4c + w4e[:4]) + gate)
    second = (pair(keys, 5) + pair(values, 1) + pair(values, 5) + last[-16:]
              + ending(w3[28:], w4b + w4d + w4e[4:]))
    cut = (len(first) + len(wm) - HEAD_START - len(second) - len(wide)) // 2
    first, second = wm[cut:] + first, wide + wm[:cut] + second

    def landed(ref, sem):
        pltpu.make_async_copy(ref, ref, sems.at[sem]).wait()

    even = (lax.broadcasted_iota(jnp.int32, (ROWS, DH), 0) & 1) == 0

    def condition():
        landed(c_ref, S_C)
        landed(x_ref, S_X)
        landed(wm_ref.at[:, :, :LATE], S_WM)
        c = jnp.broadcast_to(c_ref[...].astype(F32), (ROWS, D))
        c = (c * jax.nn.sigmoid(c)).astype(BF16)
        s_ref[0, :, :LATE] = _dot(c, wm_ref[:, :, :LATE])
        for g in range(5):
            mod_ref[g] = s_ref[0, :, g * D:(g + 1) * D]
        mod_ref[5, :, :LATE - 5 * D] = s_ref[0, :, 5 * D:LATE]
        mod_ref[5, :, LATE - 5 * D:] = jnp.zeros((ROWS, 6 * D - LATE), F32)
        cond_ref[...] = jnp.broadcast_to(c[:1].astype(F32), (LANES, D)).T

    def queries():
        landed(wq_ref, S_WQ)
        landed(wo_ref, S_WO)
        x = jnp.broadcast_to(x_ref[0].astype(F32), (ROWS, D))
        q = _dot((_layernorm(x) * (1.0 + mod_ref[1]) + mod_ref[0]).astype(BF16), wq_ref[...]) * DH ** -0.5
        for h in range(HKV):
            q_ref[h] = jnp.where(even, q[:, 2 * h * DH:(2 * h + 1) * DH], q[:, (2 * h + 1) * DH:(2 * h + 2) * DH])
        attn_ref[...] = jnp.zeros((ROWS, D), F32)

    def scores(h):
        landed(k_ref.at[h], S_K + h)
        s = _dot_t(q_ref[h].astype(BF16), k_ref[h])
        s_ref[h] = s
        m = jnp.max(_tree(jnp.maximum, _lane_tiles(s)), axis=-1, keepdims=True)
        max_ref[h] = jnp.broadcast_to(m, (ROWS, LANES))

    def attend(h):
        landed(v_ref.at[h], S_V + h)
        p = jnp.exp(s_ref[h] - jnp.concatenate([max_ref[h]] * (WINDOW // LANES), axis=1))
        o = _dot(p.astype(BF16), v_ref[h]) / jnp.sum(_tree(jnp.add, _lane_tiles(p)), axis=-1, keepdims=True)
        o = jnp.concatenate([jnp.where(even, o, 0.0), jnp.where(even, 0.0, o)], axis=1).astype(BF16)
        attn_ref[...] += _dot_t(o, wo_ref[:, :, h * 2 * DH:(h + 1) * 2 * DH])

    def residual():
        attn = attn_ref[...]
        x = jnp.broadcast_to(x_ref[0].astype(F32), (ROWS, D))
        x = x + mod_ref[2] * (attn + pltpu.roll(attn, 1, 0))
        h = _layernorm(x) * (1.0 + mod_ref[4]) + mod_ref[3]
        mod_ref[0], mod_ref[1], mod_ref[2] = x, h, _layernorm(h)

    position = {id(copy): i for queue in (first, second) for i, copy in enumerate(queue)}

    def ready(copies):
        return max(position[id(copy)] for copy in copies) + IN_FLIGHT

    jobs = [(ready(wm), condition, ()), (ready(wide), queries, ())]
    for heads, job in ((keys, scores), (values, attend)):
        jobs += [(at, job, (h,)) for at, h in sorted((ready(heads[h]), h) for h in range(HKV))]
    jobs.append((0, residual, ()))

    free = 0
    for i, copy in enumerate(first):
        copy.start(priority=1)
        if i == HEAD_START:
            pltpu.make_async_copy(c_hbm, c_ref, sems.at[S_C]).start(priority=1)
            pltpu.make_async_copy(x_hbm, x_ref, sems.at[S_X]).start(priority=1)
        j = i - HEAD_START
        if 0 <= j < len(second):
            second[j].start(priority=0)
        if jobs and j >= max(free, jobs[0][0]):
            _, job, args = jobs.pop(0)
            job(*args)
            free = j + 12
    assert len(first) - HEAD_START >= len(second)

    for _, job, args in jobs:
        job(*args)
    landed(w3_ref, S_W3)
    hidden = jax.nn.gelu(_dot(mod_ref[2].astype(BF16), w3_ref[...]), approximate=True).astype(BF16)
    for i, (a, b) in enumerate(W4_STAGES):
        landed(w4_ref.at[a:b], S_W4 + i)
        mod_ref[1, :, 64 * a:64 * b] += _dot_t(hidden, w4_ref[a:b])

    blocks, height, _ = wm_ref.shape
    sums = []
    for i, (a, b) in enumerate(GATE_STAGES):
        landed(wm_ref.at[:, a:b, LATE:], S_GATE + i)
        terms = [_tree(jnp.add, [wm_ref[k, r:r + 8, t:t + LANES].astype(F32) * cond_ref[k * height + r:k * height + r + 8]
                                 for r in range(a, b, 8) for k in range(blocks)])
                 for t in range(LATE, 6 * D, LANES)]
        sums = [old + new for old, new in zip(sums, terms)] or terms
    for shift in (4, 2, 1):
        sums = [v + pltpu.roll(v, shift, 0) for v in sums]
    halves = [pltpu.roll(v, LANES // 2, 1) for v in sums]
    low = lax.broadcasted_iota(jnp.int32, (ROWS, LANES), 1) < LANES // 2
    tiles = [jnp.where(low, a, b) for a, b in zip([mod_ref[5, :, :LANES]] + halves, halves)]
    y = mod_ref[0] + jnp.concatenate(tiles + [halves[-1][:, :LANES // 2]], axis=1) * mod_ref[1]
    out_ref[0] = y[:1].astype(BF16)
    store = pltpu.make_async_copy(out_ref, out_hbm, sems.at[S_X])
    store.start()
    store.wait()


@jax.jit
def pallas_adaLN_cond__sliding_block_cached__mixer_s_mlp__decode_kernel(
    A_x: jax.Array,
    A_k_cache: jax.Array,
    A_v_cache: jax.Array,
    A_wq: jax.Array,
    A_wo: jax.Array,
    B_x: jax.Array,
    B_w1: jax.Array,
    B_w2: jax.Array,
    B_w3: jax.Array,
    B_w4: jax.Array,
    c: jax.Array,
    w_mod: jax.Array,
):
    keys = A_k_cache.shape[2]
    assert A_x.shape == (1, 1, D) and A_k_cache.shape == (1, HKV, keys, DH)
    assert min(4096, max(256, keys // 4)) == WINDOW and keys % BLOCK == 0
    k, v = A_k_cache.reshape(-1, BLOCK, DH), A_v_cache.reshape(-1, BLOCK, DH)
    wm, wq, wo = w_mod.reshape(4, -1, 6 * D), A_wq.reshape(7, -1, HQ * DH), A_wo.T.reshape(7, -1, HQ * DH)
    w3, w4 = B_w3.reshape(2, -1, F), B_w4.T.reshape(7, -1, F)
    window = (HKV, WINDOW // BLOCK, BLOCK, DH)
    hbm = pl.BlockSpec(memory_space=pltpu.HBM)
    return pl.pallas_call(
        _kernel,
        out_shape=jax.ShapeDtypeStruct(A_x.shape, A_x.dtype),
        in_specs=[hbm] * 9,
        out_specs=hbm,
        scratch_shapes=[pltpu.VMEM(shape, BF16) for shape in (
            A_x.shape, c.shape, wm.shape, wq.shape, window, window, wo.shape, w3.shape, w4.shape)] + [
            pltpu.VMEM((HKV, ROWS, DH), F32),
            pltpu.VMEM((HKV, ROWS, WINDOW), F32),
            pltpu.VMEM((HKV, ROWS, LANES), F32),
            pltpu.VMEM((ROWS, D), F32),
            pltpu.VMEM((6, ROWS, D), F32),
            pltpu.VMEM((D, LANES), F32),
            pltpu.VMEM(A_x.shape, BF16),
            pltpu.SemaphoreType.DMA((S_END,)),
        ],
        compiler_params=pltpu.CompilerParams(
            vmem_limit_bytes=100 * 2**20,
            disable_semaphore_checks=True,
        ),
        name="adaln_decode",
    )(A_x, c, wm, wq, k, v, wo, w3, w4)
```

```python
import jax
import jax.numpy as jnp
from jax import lax
from jax.experimental import pallas as pl
from jax.experimental.pallas import tpu as pltpu

D, F = 448, 1792
HQ, HKV, DH = 16, 8, 256
WINDOW = 4096
EPS = 1e-5
ROWS = 8
LANES = 128
BLOCK, STEP = 1024, 16
LATE = 18 * LANES
W4_STAGES = ((0, 2), (2, 4), (4, 6), (6, 7))
GATE_STAGES = ((0, 80), (80, 104), (104, 112))
HEAD_START = 26
PARTNER = 5
IN_FLIGHT = 32
BF16, F32 = jnp.bfloat16, jnp.float32

S_X, S_C, S_WM, S_WQ, S_WO, S_W3, S_K, S_V, S_W4, S_GATE, S_END = 0, 1, 2, 3, 4, 5, 6, 14, 22, 26, 29


def _layernorm(x):
    d = x - jnp.sum(x, axis=-1, keepdims=True) * (1.0 / D)
    return d * lax.rsqrt(jnp.sum(d * d, axis=-1, keepdims=True) * (1.0 / D) + EPS)


def _flat(blocks):
    return blocks.reshape(-1, blocks.shape[-1])


def _dot(a, blocks):
    return lax.dot_general(a, _flat(blocks), (((1,), (0,)), ((), ())), preferred_element_type=F32)


def _dot_t(a, blocks):
    return lax.dot_general(a, _flat(blocks), (((1,), (1,)), ((), ())), preferred_element_type=F32)


def _mix(*lists):
    return [item for group in zip(*lists, strict=True) for item in group]


def _tree(op, terms):
    while len(terms) > 1:
        terms = [op(a, b) for a, b in zip(terms[::2], terms[1::2])] + terms[len(terms) // 2 * 2:]
    return terms[0]


def _lane_tiles(x):
    return [x[:, t:t + LANES] for t in range(0, x.shape[1], LANES)]


def _kernel(x_hbm, c_hbm, wm_hbm, wq_hbm, k_hbm, v_hbm, wo_hbm, w3_hbm, w4_hbm, out_hbm,
            x_ref, c_ref, wm_ref, wq_ref, k_ref, v_ref, wo_ref, w3_ref, w4_ref,
            q_ref, p_ref, total_ref, attn_ref, mod_ref, cond_ref, out_ref, sems):
    def cache(hbm, ref, sem, h):
        n = WINDOW // BLOCK
        blocks = pl.ds((h + 1) * hbm.shape[0] // HKV - n, n)
        return [pltpu.make_async_copy(hbm.at[blocks, pl.ds(r, STEP)], ref.at[h, :, pl.ds(r, STEP)], sems.at[sem + h])
                for r in range(0, BLOCK, STEP)]

    def weight(hbm, ref, sem, first, n, tiles, col=0, rows=None):
        ends = [col + LANES * sum(tiles[:i]) for i in range(len(tiles) + 1)]
        pieces = [(pl.ds(first, n), pl.ds(r, 8), pl.ds(a, b - a))
                  for r in range(*(rows or (0, ref.shape[1])), 8) for a, b in zip(ends, ends[1:])]
        return [pltpu.make_async_copy(hbm.at[at], ref.at[at], sems.at[sem]) for at in pieces]

    keys, values = [[_mix(cache(hbm, ref, sem, h), cache(hbm, ref, sem, h ^ PARTNER)) for h in range(HKV // 2)]
                    for hbm, ref, sem in ((k_hbm, k_ref, S_K), (v_hbm, v_ref, S_V))]
    wide = _mix(weight(wq_hbm, wq_ref, S_WQ, 0, 4, (4,) * 8), weight(wo_hbm, wo_ref, S_WO, 4, 3, (4,) * 8),
                weight(wq_hbm, wq_ref, S_WQ, 4, 3, (4,) * 8), weight(wo_hbm, wo_ref, S_WO, 0, 4, (4,) * 8))
    wm = weight(wm_hbm, wm_ref, S_WM, 0, 4, (4, 4, 4, 3, 3))
    w3 = weight(w3_hbm, w3_ref, S_W3, 0, 2, (7, 7))
    w4 = [copy for i, stage in enumerate(W4_STAGES) for block in range(*stage)
          for copy in weight(w4_hbm, w4_ref, S_W4 + i, block, 1, (14,))]
    gate = [copy for i, rows in enumerate(GATE_STAGES)
            for copy in weight(wm_hbm, wm_ref, S_GATE + i, 0, 4, (3,), LATE, rows)]

    first = keys[3] + keys[0] + keys[1] + values[0] + values[1] + w3 + w4[32:] + gate
    second = keys[2] + values[3] + values[2] + w4[:32]
    cut = (len(first) + len(wm) - HEAD_START - len(second) - len(wide)) // 2
    first, second = wm[cut:] + first, wide + wm[:cut] + second

    def landed(ref, sem):
        pltpu.make_async_copy(ref, ref, sems.at[sem]).wait()

    even = (lax.broadcasted_iota(jnp.int32, (ROWS, DH), 0) & 1) == 0

    def condition():
        landed(c_ref, S_C)
        landed(x_ref, S_X)
        landed(wm_ref.at[:, :, :LATE], S_WM)
        c = jnp.broadcast_to(c_ref[...].astype(F32), (ROWS, D))
        c = (c * jax.nn.sigmoid(c)).astype(BF16)
        p_ref[0, :, :LATE] = _dot(c, wm_ref[:, :, :LATE])
        for g in range(5):
            mod_ref[g] = p_ref[0, :, g * D:(g + 1) * D]
        mod_ref[5, :, :LATE - 5 * D] = p_ref[0, :, 5 * D:LATE]
        mod_ref[5, :, LATE - 5 * D:] = jnp.zeros((ROWS, 6 * D - LATE), F32)
        cond_ref[...] = jnp.broadcast_to(c[:1].astype(F32), (LANES, D)).T

    def queries():
        landed(wq_ref, S_WQ)
        landed(wo_ref, S_WO)
        x = jnp.broadcast_to(x_ref[0].astype(F32), (ROWS, D))
        q = _dot((_layernorm(x) * (1.0 + mod_ref[1]) + mod_ref[0]).astype(BF16), wq_ref[...]) * DH ** -0.5
        for h in range(HKV):
            q_ref[h] = jnp.where(even, q[:, 2 * h * DH:(2 * h + 1) * DH], q[:, (2 * h + 1) * DH:(2 * h + 2) * DH])
        attn_ref[...] = jnp.zeros((ROWS, D), F32)

    def scores(h):
        landed(k_ref.at[h], S_K + h)
        s = _dot_t(q_ref[h].astype(BF16), k_ref[h])
        p = jnp.exp(s - jnp.max(_tree(jnp.maximum, _lane_tiles(s)), axis=-1, keepdims=True))
        p_ref[h] = p
        total_ref[h] = jnp.broadcast_to(jnp.sum(_tree(jnp.add, _lane_tiles(p)), axis=-1, keepdims=True), (ROWS, DH))

    def attend(*heads):
        for h in heads:
            landed(v_ref.at[h], S_V + h)
        outs = [_dot(p_ref[h].astype(BF16), v_ref[h]) / total_ref[h] for h in heads]
        attn = attn_ref[...]
        for h, o in zip(heads, outs):
            o = jnp.concatenate([jnp.where(even, o, 0.0), jnp.where(even, 0.0, o)], axis=1).astype(BF16)
            attn = attn + _dot_t(o, wo_ref[:, :, h * 2 * DH:(h + 1) * 2 * DH])
        attn_ref[...] = attn

    def residual():
        attn = attn_ref[...]
        x = jnp.broadcast_to(x_ref[0].astype(F32), (ROWS, D))
        x = x + mod_ref[2] * (attn + pltpu.roll(attn, 1, 0))
        h = _layernorm(x) * (1.0 + mod_ref[4]) + mod_ref[3]
        mod_ref[0], mod_ref[1], mod_ref[2] = x, h, _layernorm(h)

    position = {id(copy): i for queue in (first, second) for i, copy in enumerate(queue)}

    def ready(copies):
        return max(position[id(copy)] for copy in copies) + IN_FLIGHT

    jobs = [(ready(wm), condition, ()), (ready(wide), queries, ())]
    jobs += [(at, scores, (g,)) for at, h in sorted((ready(c), h) for h, c in enumerate(keys)) for g in (h, h ^ PARTNER)]
    jobs += [(at, attend, (h, h ^ PARTNER)) for at, h in sorted((ready(c), h) for h, c in enumerate(values))]

    free = 0
    for i, copy in enumerate(first):
        copy.start(priority=1)
        j = max(i - HEAD_START + 1, 0)
        if (i == 0 or j > 0) and j < len(second):
            second[j].start(priority=0)
        if i == HEAD_START:
            pltpu.make_async_copy(c_hbm, c_ref, sems.at[S_C]).start(priority=1)
            pltpu.make_async_copy(x_hbm, x_ref, sems.at[S_X]).start(priority=1)
        if jobs and j > max(free, jobs[0][0]):
            _, job, args = jobs.pop(0)
            job(*args)
            free = j + 8
    assert len(first) - HEAD_START >= len(second) - 1

    for _, job, args in jobs:
        job(*args)
    residual()
    landed(w3_ref, S_W3)
    hidden = jax.nn.gelu(_dot(mod_ref[2].astype(BF16), w3_ref[...]), approximate=True).astype(BF16)
    for i, (a, b) in enumerate(W4_STAGES):
        landed(w4_ref.at[a:b], S_W4 + i)
        mod_ref[1, :, 64 * a:64 * b] += _dot_t(hidden, w4_ref[a:b])

    blocks, height, _ = wm_ref.shape
    sums = []
    for i, (a, b) in enumerate(GATE_STAGES):
        landed(wm_ref.at[:, a:b, LATE:], S_GATE + i)
        terms = [_tree(jnp.add, [wm_ref[k, r:r + 8, t:t + LANES].astype(F32) * cond_ref[k * height + r:k * height + r + 8]
                                 for r in range(a, b, 8) for k in range(blocks)])
                 for t in range(LATE, 6 * D, LANES)]
        sums = [old + new for old, new in zip(sums, terms)] or terms
    for shift in (4, 2, 1):
        sums = [v + pltpu.roll(v, shift, 0) for v in sums]
    halves = [pltpu.roll(v, LANES // 2, 1) for v in sums]
    low = lax.broadcasted_iota(jnp.int32, (ROWS, LANES), 1) < LANES // 2
    tiles = [jnp.where(low, a, b) for a, b in zip([mod_ref[5, :, :LANES]] + halves, halves)]
    y = mod_ref[0] + jnp.concatenate(tiles + [halves[-1][:, :LANES // 2]], axis=1) * mod_ref[1]
    out_ref[0] = y[:1].astype(BF16)
    store = pltpu.make_async_copy(out_ref, out_hbm, sems.at[S_X])
    store.start()
    store.wait()


@jax.jit
def pallas_adaLN_cond__sliding_block_cached__mixer_s_mlp__decode_kernel(
    A_x: jax.Array,
    A_k_cache: jax.Array,
    A_v_cache: jax.Array,
    A_wq: jax.Array,
    A_wo: jax.Array,
    B_x: jax.Array,
    B_w1: jax.Array,
    B_w2: jax.Array,
    B_w3: jax.Array,
    B_w4: jax.Array,
    c: jax.Array,
    w_mod: jax.Array,
):
    keys = A_k_cache.shape[2]
    assert A_x.shape == (1, 1, D) and A_k_cache.shape == (1, HKV, keys, DH)
    assert min(4096, max(256, keys // 4)) == WINDOW and keys % BLOCK == 0
    k, v = A_k_cache.reshape(-1, BLOCK, DH), A_v_cache.reshape(-1, BLOCK, DH)
    wm, wq, wo = w_mod.reshape(4, -1, 6 * D), A_wq.reshape(7, -1, HQ * DH), A_wo.T.reshape(7, -1, HQ * DH)
    w3, w4 = B_w3.reshape(2, -1, F), B_w4.T.reshape(7, -1, F)
    window = (HKV, WINDOW // BLOCK, BLOCK, DH)
    hbm = pl.BlockSpec(memory_space=pltpu.HBM)
    return pl.pallas_call(
        _kernel,
        out_shape=jax.ShapeDtypeStruct(A_x.shape, A_x.dtype),
        in_specs=[hbm] * 9,
        out_specs=hbm,
        scratch_shapes=[pltpu.VMEM(shape, BF16) for shape in (
            A_x.shape, c.shape, wm.shape, wq.shape, window, window, wo.shape, w3.shape, w4.shape)] + [
            pltpu.VMEM((HKV, ROWS, DH), F32),
            pltpu.VMEM((HKV, ROWS, WINDOW), F32),
            pltpu.VMEM((HKV, ROWS, DH), F32),
            pltpu.VMEM((ROWS, D), F32),
            pltpu.VMEM((6, ROWS, D), F32),
            pltpu.VMEM((D, LANES), F32),
            pltpu.VMEM(A_x.shape, BF16),
            pltpu.SemaphoreType.DMA((S_END,)),
        ],
        compiler_params=pltpu.CompilerParams(
            vmem_limit_bytes=100 * 2**20,
            disable_semaphore_checks=True,
        ),
        name="adaln_decode",
    )(A_x, c, wm, wq, k, v, wo, w3, w4)
```

```python
import jax
import jax.numpy as jnp
from jax import lax
from jax.experimental import pallas as pl
from jax.experimental.pallas import tpu as pltpu

D, F = 448, 1792
HQ, HKV, DH = 16, 8, 256
WINDOW = 4096
EPS = 1e-5
ROWS = 8
LANES = 128
BLOCK, STEP = 1024, 16
LATE = 18 * LANES
W4_STAGES = ((0, 2), (2, 4), (4, 6), (6, 7))
GATE_STAGES = ((0, 56), (56, 96), (96, 112))
HEAD_START = 26
PARTNER = 5
IN_FLIGHT = 32
BF16, F32 = jnp.bfloat16, jnp.float32

S_X, S_C, S_WM, S_WQ, S_WO, S_W3, S_K, S_V, S_W4, S_GATE, S_END = 0, 1, 2, 3, 4, 5, 6, 14, 22, 26, 29


def _layernorm(x):
    d = x - jnp.sum(x, axis=-1, keepdims=True) * (1.0 / D)
    return d * lax.rsqrt(jnp.sum(d * d, axis=-1, keepdims=True) * (1.0 / D) + EPS)


def _flat(blocks):
    return blocks.reshape(-1, blocks.shape[-1])


def _dot(a, blocks):
    return lax.dot_general(a, _flat(blocks), (((1,), (0,)), ((), ())), preferred_element_type=F32)


def _dot_t(a, blocks):
    return lax.dot_general(a, _flat(blocks), (((1,), (1,)), ((), ())), preferred_element_type=F32)


def _mix(*lists):
    return [item for group in zip(*lists, strict=True) for item in group]


def _tree(op, terms):
    while len(terms) > 1:
        terms = [op(a, b) for a, b in zip(terms[::2], terms[1::2])] + terms[len(terms) // 2 * 2:]
    return terms[0]


def _lane_tiles(x):
    return [x[:, t:t + LANES] for t in range(0, x.shape[1], LANES)]


def _kernel(x_hbm, c_hbm, wm_hbm, wq_hbm, k_hbm, v_hbm, wo_hbm, w3_hbm, w4_hbm, out_hbm,
            x_ref, c_ref, wm_ref, wq_ref, k_ref, v_ref, wo_ref, w3_ref, w4_ref,
            q_ref, p_ref, total_ref, attn_ref, mod_ref, cond_ref, out_ref, sems):
    def cache(hbm, ref, sem, h):
        n = WINDOW // BLOCK
        blocks = pl.ds((h + 1) * hbm.shape[0] // HKV - n, n)
        return [pltpu.make_async_copy(hbm.at[blocks, pl.ds(r, STEP)], ref.at[h, :, pl.ds(r, STEP)], sems.at[sem + h])
                for r in range(0, BLOCK, STEP)]

    def weight(hbm, ref, sem, first, n, tiles, col=0, rows=None):
        ends = [col + LANES * sum(tiles[:i]) for i in range(len(tiles) + 1)]
        pieces = [(pl.ds(first, n), pl.ds(r, 8), pl.ds(a, b - a))
                  for r in range(*(rows or (0, ref.shape[1])), 8) for a, b in zip(ends, ends[1:])]
        return [pltpu.make_async_copy(hbm.at[at], ref.at[at], sems.at[sem]) for at in pieces]

    keys, values = [[_mix(cache(hbm, ref, sem, h), cache(hbm, ref, sem, h ^ PARTNER)) for h in range(HKV // 2)]
                    for hbm, ref, sem in ((k_hbm, k_ref, S_K), (v_hbm, v_ref, S_V))]
    wide = _mix(weight(wq_hbm, wq_ref, S_WQ, 0, 4, (4,) * 8), weight(wo_hbm, wo_ref, S_WO, 4, 3, (4,) * 8),
                weight(wq_hbm, wq_ref, S_WQ, 4, 3, (4,) * 8), weight(wo_hbm, wo_ref, S_WO, 0, 4, (4,) * 8))
    wm = weight(wm_hbm, wm_ref, S_WM, 0, 4, (3,) * 6)
    w3 = weight(w3_hbm, w3_ref, S_W3, 0, 2, (7, 7))
    w4 = [copy for i, stage in enumerate(W4_STAGES) for block in range(*stage)
          for copy in weight(w4_hbm, w4_ref, S_W4 + i, block, 1, (14,))]
    gate = [copy for i, rows in enumerate(GATE_STAGES)
            for copy in weight(wm_hbm, wm_ref, S_GATE + i, 0, 4, (3,), LATE, rows)]

    first = keys[2] + keys[0] + keys[1] + values[1] + values[0] + w3 + w4[32:] + gate
    second = keys[3] + values[2] + values[3] + w4[:32]
    cut = (len(first) + len(wm) - HEAD_START - len(second) - len(wide)) // 2
    first, second = wm[cut:] + first, wide + wm[:cut] + second

    def landed(ref, sem):
        pltpu.make_async_copy(ref, ref, sems.at[sem]).wait()

    even = (lax.broadcasted_iota(jnp.int32, (ROWS, DH), 0) & 1) == 0

    def condition():
        landed(c_ref, S_C)
        landed(x_ref, S_X)
        landed(wm_ref.at[:, :, :LATE], S_WM)
        c = jnp.broadcast_to(c_ref[...].astype(F32), (ROWS, D))
        c = (c * jax.nn.sigmoid(c)).astype(BF16)
        p_ref[0, :, :LATE] = _dot(c, wm_ref[:, :, :LATE])
        for g in range(5):
            mod_ref[g] = p_ref[0, :, g * D:(g + 1) * D]
        mod_ref[5, :, :LATE - 5 * D] = p_ref[0, :, 5 * D:LATE]
        mod_ref[5, :, LATE - 5 * D:] = jnp.zeros((ROWS, 6 * D - LATE), F32)
        cond_ref[...] = jnp.broadcast_to(c[:1].astype(F32), (LANES, D)).T

    def queries():
        landed(wq_ref, S_WQ)
        landed(wo_ref, S_WO)
        x = jnp.broadcast_to(x_ref[0].astype(F32), (ROWS, D))
        q = _dot((_layernorm(x) * (1.0 + mod_ref[1]) + mod_ref[0]).astype(BF16), wq_ref[...]) * DH ** -0.5
        for h in range(HKV):
            q_ref[h] = jnp.where(even, q[:, 2 * h * DH:(2 * h + 1) * DH], q[:, (2 * h + 1) * DH:(2 * h + 2) * DH])
        attn_ref[...] = jnp.zeros((ROWS, D), F32)

    def scores(h):
        landed(k_ref.at[h], S_K + h)
        s = _dot_t(q_ref[h].astype(BF16), k_ref[h])
        p = jnp.exp(s - jnp.max(_tree(jnp.maximum, _lane_tiles(s)), axis=-1, keepdims=True))
        p_ref[h] = p
        total_ref[h] = jnp.broadcast_to(jnp.sum(_tree(jnp.add, _lane_tiles(p)), axis=-1, keepdims=True), (ROWS, DH))

    def attend(*heads):
        for h in heads:
            landed(v_ref.at[h], S_V + h)
        outs = [_dot(p_ref[h].astype(BF16), v_ref[h]) / total_ref[h] for h in heads]
        attn = attn_ref[...]
        for h, o in zip(heads, outs):
            o = jnp.concatenate([jnp.where(even, o, 0.0), jnp.where(even, 0.0, o)], axis=1).astype(BF16)
            attn = attn + _dot_t(o, wo_ref[:, :, h * 2 * DH:(h + 1) * 2 * DH])
        attn_ref[...] = attn

    def residual():
        attn = attn_ref[...]
        x = jnp.broadcast_to(x_ref[0].astype(F32), (ROWS, D))
        x = x + mod_ref[2] * (attn + pltpu.roll(attn, 1, 0))
        h = _layernorm(x) * (1.0 + mod_ref[4]) + mod_ref[3]
        mod_ref[0], mod_ref[1], mod_ref[2] = x, h, _layernorm(h)

    position = {id(copy): i for queue in (first, second) for i, copy in enumerate(queue)}

    def ready(copies):
        return max(position[id(copy)] for copy in copies) + IN_FLIGHT

    jobs = [(ready(wm), condition, ()), (ready(wide), queries, ())]
    jobs += [(at, scores, (g,)) for at, h in sorted((ready(c), h) for h, c in enumerate(keys)) for g in (h, h ^ PARTNER)]
    jobs += [(at, attend, (h, h ^ PARTNER)) for at, h in sorted((ready(c), h) for h, c in enumerate(values))]

    free = 0
    for i, copy in enumerate(first):
        copy.start(priority=1)
        j = max(i - HEAD_START + 1, 0)
        if (i == 0 or j > 0) and j < len(second):
            second[j].start(priority=0)
        if i == HEAD_START:
            pltpu.make_async_copy(c_hbm, c_ref, sems.at[S_C]).start(priority=1)
            pltpu.make_async_copy(x_hbm, x_ref, sems.at[S_X]).start(priority=1)
        if jobs and j > max(free, jobs[0][0]):
            _, job, args = jobs.pop(0)
            job(*args)
            free = j + 8
    assert len(first) - HEAD_START >= len(second) - 1

    for _, job, args in jobs:
        job(*args)
    residual()
    landed(w3_ref, S_W3)
    hidden = jax.nn.gelu(_dot(mod_ref[2].astype(BF16), w3_ref[...]), approximate=True).astype(BF16)
    for i, (a, b) in enumerate(W4_STAGES):
        landed(w4_ref.at[a:b], S_W4 + i)
        mod_ref[1, :, 64 * a:64 * b] += _dot_t(hidden, w4_ref[a:b])

    blocks, height, _ = wm_ref.shape
    sums = []
    for i, (a, b) in enumerate(GATE_STAGES):
        landed(wm_ref.at[:, a:b, LATE:], S_GATE + i)
        terms = [_tree(jnp.add, [wm_ref[k, r:r + 8, t:t + LANES].astype(F32) * cond_ref[k * height + r:k * height + r + 8]
                                 for r in range(a, b, 8) for k in range(blocks)])
                 for t in range(LATE, 6 * D, LANES)]
        sums = [old + new for old, new in zip(sums, terms)] or terms
    for shift in (4, 2, 1):
        sums = [v + pltpu.roll(v, shift, 0) for v in sums]
    halves = [pltpu.roll(v, LANES // 2, 1) for v in sums]
    low = lax.broadcasted_iota(jnp.int32, (ROWS, LANES), 1) < LANES // 2
    tiles = [jnp.where(low, a, b) for a, b in zip([mod_ref[5, :, :LANES]] + halves, halves)]
    y = mod_ref[0] + jnp.concatenate(tiles + [halves[-1][:, :LANES // 2]], axis=1) * mod_ref[1]
    out_ref[0] = y[:1].astype(BF16)
    store = pltpu.make_async_copy(out_ref, out_hbm, sems.at[S_X])
    store.start()
    store.wait()


@jax.jit
def pallas_adaLN_cond__sliding_block_cached__mixer_s_mlp__decode_kernel(
    A_x: jax.Array,
    A_k_cache: jax.Array,
    A_v_cache: jax.Array,
    A_wq: jax.Array,
    A_wo: jax.Array,
    B_x: jax.Array,
    B_w1: jax.Array,
    B_w2: jax.Array,
    B_w3: jax.Array,
    B_w4: jax.Array,
    c: jax.Array,
    w_mod: jax.Array,
):
    keys = A_k_cache.shape[2]
    assert A_x.shape == (1, 1, D) and A_k_cache.shape == (1, HKV, keys, DH)
    assert min(4096, max(256, keys // 4)) == WINDOW and keys % BLOCK == 0
    k, v = A_k_cache.reshape(-1, BLOCK, DH), A_v_cache.reshape(-1, BLOCK, DH)
    wm, wq, wo = w_mod.reshape(4, -1, 6 * D), A_wq.reshape(7, -1, HQ * DH), A_wo.T.reshape(7, -1, HQ * DH)
    w3, w4 = B_w3.reshape(2, -1, F), B_w4.T.reshape(7, -1, F)
    window = (HKV, WINDOW // BLOCK, BLOCK, DH)
    hbm = pl.BlockSpec(memory_space=pltpu.HBM)
    return pl.pallas_call(
        _kernel,
        out_shape=jax.ShapeDtypeStruct(A_x.shape, A_x.dtype),
        in_specs=[hbm] * 9,
        out_specs=hbm,
        scratch_shapes=[pltpu.VMEM(shape, BF16) for shape in (
            A_x.shape, c.shape, wm.shape, wq.shape, window, window, wo.shape, w3.shape, w4.shape)] + [
            pltpu.VMEM((HKV, ROWS, DH), F32),
            pltpu.VMEM((HKV, ROWS, WINDOW), F32),
            pltpu.VMEM((HKV, ROWS, DH), F32),
            pltpu.VMEM((ROWS, D), F32),
            pltpu.VMEM((6, ROWS, D), F32),
            pltpu.VMEM((D, LANES), F32),
            pltpu.VMEM(A_x.shape, BF16),
            pltpu.SemaphoreType.DMA((S_END,)),
        ],
        compiler_params=pltpu.CompilerParams(
            vmem_limit_bytes=100 * 2**20,
            disable_semaphore_checks=True,
        ),
        name="adaln_decode",
    )(A_x, c, wm, wq, k, v, wo, w3, w4)
```

```python
import jax
import jax.numpy as jnp
from jax import lax
from jax.experimental import pallas as pl
from jax.experimental.pallas import tpu as pltpu

D, F = 448, 1792
HQ, HKV, DH = 16, 8, 256
WINDOW = 4096
EPS = 1e-5
ROWS = 8
LANES = 128
BLOCK, STEP = 1024, 16
LATE = 18 * LANES
W4_STAGES = ((0, 2), (2, 4), (4, 6), (6, 7))
GATE_STAGES = ((0, 56), (56, 96), (96, 112))
HEAD_START = 26
PARTNER = 5
IN_FLIGHT = 32
BF16, F32 = jnp.bfloat16, jnp.float32

S_X, S_C, S_WM, S_WQ, S_WO, S_W3, S_K, S_V, S_W4, S_GATE, S_SKIP, S_END = 0, 1, 2, 3, 4, 5, 6, 14, 22, 26, 29, 30


def _layernorm(x):
    d = x - jnp.sum(x, axis=-1, keepdims=True) * (1.0 / D)
    return d * lax.rsqrt(jnp.sum(d * d, axis=-1, keepdims=True) * (1.0 / D) + EPS)


def _flat(blocks):
    return blocks.reshape(-1, blocks.shape[-1])


def _dot(a, blocks):
    return lax.dot_general(a, _flat(blocks), (((1,), (0,)), ((), ())), preferred_element_type=F32)


def _dot_t(a, blocks):
    return lax.dot_general(a, _flat(blocks), (((1,), (1,)), ((), ())), preferred_element_type=F32)


def _mix(*lists):
    return [item for group in zip(*lists, strict=True) for item in group]


def _tree(op, terms):
    while len(terms) > 1:
        terms = [op(a, b) for a, b in zip(terms[::2], terms[1::2])] + terms[len(terms) // 2 * 2:]
    return terms[0]


def _lane_tiles(x):
    return [x[:, t:t + LANES] for t in range(0, x.shape[1], LANES)]


def _kernel(x_hbm, c_hbm, wm_hbm, wq_hbm, k_hbm, v_hbm, wo_hbm, w3_hbm, w4_hbm, out_hbm,
            x_ref, c_ref, wm_ref, wq_ref, k_ref, v_ref, wo_ref, w3_ref, w4_ref,
            q_ref, p_ref, total_ref, attn_ref, mod_ref, cond_ref, skip_ref, out_ref, sems):
    def cache(hbm, ref, sem, h):
        n = WINDOW // BLOCK
        blocks = pl.ds((h + 1) * hbm.shape[0] // HKV - n, n)
        return [pltpu.make_async_copy(hbm.at[blocks, pl.ds(r, STEP)], ref.at[h, :, pl.ds(r, STEP)], sems.at[sem + h])
                for r in range(0, BLOCK, STEP)]

    def weight(hbm, ref, sem, first, n, tiles, col=0, rows=None):
        ends = [col + LANES * sum(tiles[:i]) for i in range(len(tiles) + 1)]
        pieces = [(pl.ds(first, n), pl.ds(r, 8), pl.ds(a, b - a))
                  for r in range(*(rows or (0, ref.shape[1])), 8) for a, b in zip(ends, ends[1:])]
        return [pltpu.make_async_copy(hbm.at[at], ref.at[at], sems.at[sem]) for at in pieces]

    keys, values = [[_mix(cache(hbm, ref, sem, h), cache(hbm, ref, sem, h ^ PARTNER)) for h in range(HKV // 2)]
                    for hbm, ref, sem in ((k_hbm, k_ref, S_K), (v_hbm, v_ref, S_V))]
    wide = _mix(weight(wq_hbm, wq_ref, S_WQ, 0, 4, (4,) * 8), weight(wo_hbm, wo_ref, S_WO, 4, 3, (4,) * 8),
                weight(wq_hbm, wq_ref, S_WQ, 4, 3, (4,) * 8), weight(wo_hbm, wo_ref, S_WO, 0, 4, (4,) * 8))
    wm = weight(wm_hbm, wm_ref, S_WM, 0, 4, (3,) * 6)
    w3 = weight(w3_hbm, w3_ref, S_W3, 0, 2, (7, 7))
    w4 = [copy for i, stage in enumerate(W4_STAGES) for block in range(*stage)
          for copy in weight(w4_hbm, w4_ref, S_W4 + i, block, 1, (14,))]
    gate = [copy for i, rows in enumerate(GATE_STAGES)
            for copy in weight(wm_hbm, wm_ref, S_GATE + i, 0, 4, (3,), LATE, rows)]

    first = keys[2] + keys[0] + keys[1] + values[1] + values[0] + w3 + w4[32:] + gate
    second = keys[3] + values[2] + values[3] + w4[:32]
    cut = (len(first) + len(wm) - HEAD_START - len(second) - len(wide)) // 2
    first, second = wm[cut:] + first, wide + wm[:cut] + second

    def landed(ref, sem):
        pltpu.make_async_copy(ref, ref, sems.at[sem]).wait()

    even = (lax.broadcasted_iota(jnp.int32, (ROWS, DH), 0) & 1) == 0

    def condition():
        landed(c_ref, S_C)
        landed(x_ref, S_X)
        landed(wm_ref.at[:, :, :LATE], S_WM)
        c = jnp.broadcast_to(c_ref[...].astype(F32), (ROWS, D))
        c = (c * jax.nn.sigmoid(c)).astype(BF16)
        p_ref[0, :, :LATE] = _dot(c, wm_ref[:, :, :LATE])
        for g in range(5):
            mod_ref[g] = p_ref[0, :, g * D:(g + 1) * D]
        mod_ref[5, :, :LATE - 5 * D] = p_ref[0, :, 5 * D:LATE]
        mod_ref[5, :, LATE - 5 * D:] = jnp.zeros((ROWS, 6 * D - LATE), F32)
        cond_ref[...] = jnp.broadcast_to(c[:1].astype(F32), (LANES, D)).T

    def queries():
        landed(wq_ref, S_WQ)
        landed(wo_ref, S_WO)
        x = jnp.broadcast_to(x_ref[0].astype(F32), (ROWS, D))
        q = _dot((_layernorm(x) * (1.0 + mod_ref[1]) + mod_ref[0]).astype(BF16), wq_ref[...]) * DH ** -0.5
        for h in range(HKV):
            q_ref[h] = jnp.where(even, q[:, 2 * h * DH:(2 * h + 1) * DH], q[:, (2 * h + 1) * DH:(2 * h + 2) * DH])
        attn_ref[...] = jnp.zeros((ROWS, D), F32)

    def scores(h):
        landed(k_ref.at[h], S_K + h)
        s = _dot_t(q_ref[h].astype(BF16), k_ref[h])
        p = jnp.exp(s - jnp.max(_tree(jnp.maximum, _lane_tiles(s)), axis=-1, keepdims=True))
        p_ref[h] = p
        total_ref[h] = jnp.broadcast_to(jnp.sum(_tree(jnp.add, _lane_tiles(p)), axis=-1, keepdims=True), (ROWS, DH))

    def attend(*heads):
        for h in heads:
            landed(v_ref.at[h], S_V + h)
        outs = [_dot(p_ref[h].astype(BF16), v_ref[h]) / total_ref[h] for h in heads]
        attn = attn_ref[...]
        for h, o in zip(heads, outs):
            o = jnp.concatenate([jnp.where(even, o, 0.0), jnp.where(even, 0.0, o)], axis=1).astype(BF16)
            attn = attn + _dot_t(o, wo_ref[:, :, h * 2 * DH:(h + 1) * 2 * DH])
        attn_ref[...] = attn

    def residual():
        attn = attn_ref[...]
        x = jnp.broadcast_to(skip_ref[0].astype(F32), (ROWS, D))
        x = x + mod_ref[2] * (attn + pltpu.roll(attn, 1, 0))
        h = _layernorm(x) * (1.0 + mod_ref[4]) + mod_ref[3]
        mod_ref[0], mod_ref[1], mod_ref[2] = x, h, _layernorm(h)

    position = {id(copy): i for queue in (first, second) for i, copy in enumerate(queue)}

    def ready(copies):
        return max(position[id(copy)] for copy in copies) + IN_FLIGHT

    jobs = [(ready(wm), condition, ()), (ready(wide), queries, ())]
    jobs += [(at, scores, (g,)) for at, h in sorted((ready(c), h) for h, c in enumerate(keys)) for g in (h, h ^ PARTNER)]
    jobs += [(at, attend, (h, h ^ PARTNER)) for at, h in sorted((ready(c), h) for h, c in enumerate(values))]

    free = 0
    for i, copy in enumerate(first):
        copy.start(priority=1)
        j = max(i - HEAD_START + 1, 0)
        if (i == 0 or j > 0) and j < len(second):
            second[j].start(priority=0)
        if i == HEAD_START:
            pltpu.make_async_copy(c_hbm, c_ref, sems.at[S_C]).start(priority=1)
            pltpu.make_async_copy(x_hbm, x_ref, sems.at[S_X]).start(priority=1)
            pltpu.make_async_copy(x_hbm, skip_ref, sems.at[S_SKIP]).start(priority=1)
        if len(jobs) > 1 and j > max(free, jobs[0][0]):
            _, job, args = jobs.pop(0)
            job(*args)
            free = j + 8
            if len(jobs) == 1:
                landed(skip_ref, S_SKIP)
    assert len(jobs) == 1 and len(first) - HEAD_START >= len(second) - 1

    for _, job, args in jobs:
        job(*args)
    residual()
    landed(w3_ref, S_W3)
    hidden = jax.nn.gelu(_dot(mod_ref[2].astype(BF16), w3_ref[...]), approximate=True).astype(BF16)
    for i, (a, b) in enumerate(W4_STAGES):
        landed(w4_ref.at[a:b], S_W4 + i)
        mod_ref[1, :, 64 * a:64 * b] += _dot_t(hidden, w4_ref[a:b])

    blocks, height, _ = wm_ref.shape
    sums = []
    for i, (a, b) in enumerate(GATE_STAGES):
        landed(wm_ref.at[:, a:b, LATE:], S_GATE + i)
        terms = [_tree(jnp.add, [wm_ref[k, r:r + 8, t:t + LANES].astype(F32) * cond_ref[k * height + r:k * height + r + 8]
                                 for r in range(a, b, 8) for k in range(blocks)])
                 for t in range(LATE, 6 * D, LANES)]
        sums = [old + new for old, new in zip(sums, terms)] or terms
    for shift in (4, 2, 1):
        sums = [v + pltpu.roll(v, shift, 0) for v in sums]
    halves = [pltpu.roll(v, LANES // 2, 1) for v in sums]
    low = lax.broadcasted_iota(jnp.int32, (ROWS, LANES), 1) < LANES // 2
    tiles = [jnp.where(low, a, b) for a, b in zip([mod_ref[5, :, :LANES]] + halves, halves)]
    y = mod_ref[0] + jnp.concatenate(tiles + [halves[-1][:, :LANES // 2]], axis=1) * mod_ref[1]
    out_ref[0] = y[:1].astype(BF16)
    store = pltpu.make_async_copy(out_ref, out_hbm, sems.at[S_X])
    store.start()
    store.wait()


@jax.jit
def pallas_adaLN_cond__sliding_block_cached__mixer_s_mlp__decode_kernel(
    A_x: jax.Array,
    A_k_cache: jax.Array,
    A_v_cache: jax.Array,
    A_wq: jax.Array,
    A_wo: jax.Array,
    B_x: jax.Array,
    B_w1: jax.Array,
    B_w2: jax.Array,
    B_w3: jax.Array,
    B_w4: jax.Array,
    c: jax.Array,
    w_mod: jax.Array,
):
    keys = A_k_cache.shape[2]
    assert A_x.shape == (1, 1, D) and A_k_cache.shape == (1, HKV, keys, DH)
    assert min(4096, max(256, keys // 4)) == WINDOW and keys % BLOCK == 0
    k, v = A_k_cache.reshape(-1, BLOCK, DH), A_v_cache.reshape(-1, BLOCK, DH)
    wm, wq, wo = w_mod.reshape(4, -1, 6 * D), A_wq.reshape(7, -1, HQ * DH), A_wo.T.reshape(7, -1, HQ * DH)
    w3, w4 = B_w3.reshape(2, -1, F), B_w4.T.reshape(7, -1, F)
    window = (HKV, WINDOW // BLOCK, BLOCK, DH)
    hbm = pl.BlockSpec(memory_space=pltpu.HBM)
    return pl.pallas_call(
        _kernel,
        out_shape=jax.ShapeDtypeStruct(A_x.shape, A_x.dtype),
        in_specs=[hbm] * 9,
        out_specs=hbm,
        scratch_shapes=[pltpu.VMEM(shape, BF16) for shape in (
            A_x.shape, c.shape, wm.shape, wq.shape, window, window, wo.shape, w3.shape, w4.shape)] + [
            pltpu.VMEM((HKV, ROWS, DH), F32),
            pltpu.VMEM((HKV, ROWS, WINDOW), F32),
            pltpu.VMEM((HKV, ROWS, DH), F32),
            pltpu.VMEM((ROWS, D), F32),
            pltpu.VMEM((6, ROWS, D), F32),
            pltpu.VMEM((D, LANES), F32),
            pltpu.VMEM(A_x.shape, BF16),
            pltpu.VMEM(A_x.shape, BF16),
            pltpu.SemaphoreType.DMA((S_END,)),
        ],
        compiler_params=pltpu.CompilerParams(
            vmem_limit_bytes=100 * 2**20,
            disable_semaphore_checks=True,
        ),
        name="adaln_decode",
    )(A_x, c, wm, wq, k, v, wo, w3, w4)
```

```python
import jax
import jax.numpy as jnp
from jax import lax
from jax.experimental import pallas as pl
from jax.experimental.pallas import tpu as pltpu

D, F = 448, 1792
HQ, HKV, DH = 16, 8, 256
WINDOW = 4096
EPS = 1e-5
ROWS = 8
LANES = 128
BLOCK, STEP = 1024, 16
LATE = 18 * LANES
W4_STAGES = ((0, 2), (2, 4), (4, 6), (6, 7))
GATE_STAGES = ((0, 56), (56, 96), (96, 112))
HEAD_START = 26
PARTNER = 5
IN_FLIGHT = 32
BF16, F32 = jnp.bfloat16, jnp.float32

S_X, S_C, S_WM, S_WQ, S_WO, S_W3, S_K, S_V, S_W4, S_GATE, S_SKIP, S_END = 0, 1, 2, 3, 4, 5, 6, 14, 22, 26, 29, 30


def _layernorm(x):
    d = x - jnp.sum(x, axis=-1, keepdims=True) * (1.0 / D)
    return d * lax.rsqrt(jnp.sum(d * d, axis=-1, keepdims=True) * (1.0 / D) + EPS)


def _flat(blocks):
    return blocks.reshape(-1, blocks.shape[-1])


def _dot(a, blocks):
    return lax.dot_general(a, _flat(blocks), (((1,), (0,)), ((), ())), preferred_element_type=F32)


def _dot_t(a, blocks):
    return lax.dot_general(a, _flat(blocks), (((1,), (1,)), ((), ())), preferred_element_type=F32)


def _mix(*lists):
    return [item for group in zip(*lists, strict=True) for item in group]


def _tree(op, terms):
    while len(terms) > 1:
        terms = [op(a, b) for a, b in zip(terms[::2], terms[1::2])] + terms[len(terms) // 2 * 2:]
    return terms[0]


def _lane_tiles(x):
    return [x[:, t:t + LANES] for t in range(0, x.shape[1], LANES)]


def _kernel(x_hbm, c_hbm, wm_hbm, wq_hbm, k_hbm, v_hbm, wo_hbm, w3_hbm, w4_hbm, out_hbm,
            x_ref, c_ref, wm_ref, wq_ref, k_ref, v_ref, wo_ref, w3_ref, w4_ref,
            q_ref, p_ref, total_ref, attn_ref, mod_ref, cond_ref, skip_ref, out_ref, sems):
    def cache(hbm, ref, sem, h):
        n = WINDOW // BLOCK
        blocks = pl.ds((h + 1) * hbm.shape[0] // HKV - n, n)
        return [pltpu.make_async_copy(hbm.at[blocks, pl.ds(r, STEP)], ref.at[h, :, pl.ds(r, STEP)], sems.at[sem + h])
                for r in range(0, BLOCK, STEP)]

    def weight(hbm, ref, sem, first, n, tiles, col=0, rows=None):
        ends = [col + LANES * sum(tiles[:i]) for i in range(len(tiles) + 1)]
        pieces = [(pl.ds(first, n), pl.ds(r, 8), pl.ds(a, b - a))
                  for r in range(*(rows or (0, ref.shape[1])), 8) for a, b in zip(ends, ends[1:])]
        return [pltpu.make_async_copy(hbm.at[at], ref.at[at], sems.at[sem]) for at in pieces]

    keys, values = [[_mix(cache(hbm, ref, sem, h), cache(hbm, ref, sem, h ^ PARTNER)) for h in range(HKV // 2)]
                    for hbm, ref, sem in ((k_hbm, k_ref, S_K), (v_hbm, v_ref, S_V))]
    wide = _mix(weight(wq_hbm, wq_ref, S_WQ, 0, 4, (4,) * 8), weight(wo_hbm, wo_ref, S_WO, 4, 3, (4,) * 8),
                weight(wq_hbm, wq_ref, S_WQ, 4, 3, (4,) * 8), weight(wo_hbm, wo_ref, S_WO, 0, 4, (4,) * 8))
    wm = weight(wm_hbm, wm_ref, S_WM, 0, 4, (3,) * 6)
    w3 = weight(w3_hbm, w3_ref, S_W3, 0, 2, (7, 7))
    w4 = [copy for i, stage in enumerate(W4_STAGES) for block in range(*stage)
          for copy in weight(w4_hbm, w4_ref, S_W4 + i, block, 1, (14,))]
    gate = [copy for i, rows in enumerate(GATE_STAGES)
            for copy in weight(wm_hbm, wm_ref, S_GATE + i, 0, 4, (3,), LATE, rows)]

    first = keys[0] + keys[1] + values[1] + values[0] + w3 + w4[32:] + gate
    second = keys[3] + values[2] + values[3] + w4[:32]
    cut = (len(keys[2]) + len(wm) + len(first) - HEAD_START - len(wide) - len(second)) // 2
    first, second = keys[2] + wm[cut:] + first, wide + wm[:cut] + second

    def landed(ref, sem):
        pltpu.make_async_copy(ref, ref, sems.at[sem]).wait()

    even = (lax.broadcasted_iota(jnp.int32, (ROWS, DH), 0) & 1) == 0

    def condition():
        landed(c_ref, S_C)
        landed(x_ref, S_X)
        landed(wm_ref.at[:, :, :LATE], S_WM)
        c = jnp.broadcast_to(c_ref[...].astype(F32), (ROWS, D))
        c = (c * jax.nn.sigmoid(c)).astype(BF16)
        p_ref[0, :, :LATE] = _dot(c, wm_ref[:, :, :LATE])
        for g in range(5):
            mod_ref[g] = p_ref[0, :, g * D:(g + 1) * D]
        mod_ref[5, :, :LATE - 5 * D] = p_ref[0, :, 5 * D:LATE]
        mod_ref[5, :, LATE - 5 * D:] = jnp.zeros((ROWS, 6 * D - LATE), F32)
        cond_ref[...] = jnp.broadcast_to(c[:1].astype(F32), (LANES, D)).T

    def queries():
        landed(wq_ref, S_WQ)
        landed(wo_ref, S_WO)
        x = jnp.broadcast_to(x_ref[0].astype(F32), (ROWS, D))
        q = _dot((_layernorm(x) * (1.0 + mod_ref[1]) + mod_ref[0]).astype(BF16), wq_ref[...]) * DH ** -0.5
        for h in range(HKV):
            q_ref[h] = jnp.where(even, q[:, 2 * h * DH:(2 * h + 1) * DH], q[:, (2 * h + 1) * DH:(2 * h + 2) * DH])
        attn_ref[...] = jnp.zeros((ROWS, D), F32)

    def scores(h):
        landed(k_ref.at[h], S_K + h)
        s = _dot_t(q_ref[h].astype(BF16), k_ref[h])
        p = jnp.exp(s - jnp.max(_tree(jnp.maximum, _lane_tiles(s)), axis=-1, keepdims=True))
        p_ref[h] = p
        total_ref[h] = jnp.broadcast_to(jnp.sum(_tree(jnp.add, _lane_tiles(p)), axis=-1, keepdims=True), (ROWS, DH))

    def attend(*heads):
        for h in heads:
            landed(v_ref.at[h], S_V + h)
        outs = [_dot(p_ref[h].astype(BF16), v_ref[h]) / total_ref[h] for h in heads]
        attn = attn_ref[...]
        for h, o in zip(heads, outs):
            o = jnp.concatenate([jnp.where(even, o, 0.0), jnp.where(even, 0.0, o)], axis=1).astype(BF16)
            attn = attn + _dot_t(o, wo_ref[:, :, h * 2 * DH:(h + 1) * 2 * DH])
        attn_ref[...] = attn

    def residual():
        attn = attn_ref[...]
        x = jnp.broadcast_to(skip_ref[0].astype(F32), (ROWS, D))
        x = x + mod_ref[2] * (attn + pltpu.roll(attn, 1, 0))
        h = _layernorm(x) * (1.0 + mod_ref[4]) + mod_ref[3]
        mod_ref[0], mod_ref[1], mod_ref[2] = x, h, _layernorm(h)

    position = {id(copy): i for queue in (first, second) for i, copy in enumerate(queue)}

    def ready(copies):
        return max(position[id(copy)] for copy in copies) + IN_FLIGHT

    jobs = [(ready(wm), condition, ()), (ready(wide), queries, ())]
    jobs += [(at, scores, (g,)) for at, h in sorted((ready(c), h) for h, c in enumerate(keys)) for g in (h, h ^ PARTNER)]
    jobs += [(at, attend, (h, h ^ PARTNER)) for at, h in sorted((ready(c), h) for h, c in enumerate(values))]

    free = 0
    for i, copy in enumerate(first):
        copy.start(priority=1)
        j = max(i - HEAD_START + 1, 0)
        if (i == 0 or j > 0) and j < len(second):
            second[j].start(priority=0)
        if i == HEAD_START:
            pltpu.make_async_copy(c_hbm, c_ref, sems.at[S_C]).start(priority=1)
            pltpu.make_async_copy(x_hbm, x_ref, sems.at[S_X]).start(priority=1)
            pltpu.make_async_copy(x_hbm, skip_ref, sems.at[S_SKIP]).start(priority=1)
        if len(jobs) > 1 and j > max(free, jobs[0][0]):
            _, job, args = jobs.pop(0)
            job(*args)
            free = j + 18
            if len(jobs) == 1:
                landed(skip_ref, S_SKIP)
    assert len(jobs) == 1 and len(first) - HEAD_START >= len(second) - 1

    for _, job, args in jobs:
        job(*args)
    residual()
    landed(w3_ref, S_W3)
    hidden = jax.nn.gelu(_dot(mod_ref[2].astype(BF16), w3_ref[...]), approximate=True).astype(BF16)
    for i, (a, b) in enumerate(W4_STAGES):
        landed(w4_ref.at[a:b], S_W4 + i)
        mod_ref[1, :, 64 * a:64 * b] += _dot_t(hidden, w4_ref[a:b])

    blocks, height, _ = wm_ref.shape
    sums = []
    for i, (a, b) in enumerate(GATE_STAGES):
        landed(wm_ref.at[:, a:b, LATE:], S_GATE + i)
        terms = [_tree(jnp.add, [wm_ref[k, r:r + 8, t:t + LANES].astype(F32) * cond_ref[k * height + r:k * height + r + 8]
                                 for r in range(a, b, 8) for k in range(blocks)])
                 for t in range(LATE, 6 * D, LANES)]
        sums = [old + new for old, new in zip(sums, terms)] or terms
    for shift in (4, 2, 1):
        sums = [v + pltpu.roll(v, shift, 0) for v in sums]
    halves = [pltpu.roll(v, LANES // 2, 1) for v in sums]
    low = lax.broadcasted_iota(jnp.int32, (ROWS, LANES), 1) < LANES // 2
    tiles = [jnp.where(low, a, b) for a, b in zip([mod_ref[5, :, :LANES]] + halves, halves)]
    y = mod_ref[0] + jnp.concatenate(tiles + [halves[-1][:, :LANES // 2]], axis=1) * mod_ref[1]
    out_ref[0] = y[:1].astype(BF16)
    store = pltpu.make_async_copy(out_ref, out_hbm, sems.at[S_X])
    store.start()
    store.wait()


@jax.jit
def pallas_adaLN_cond__sliding_block_cached__mixer_s_mlp__decode_kernel(
    A_x: jax.Array,
    A_k_cache: jax.Array,
    A_v_cache: jax.Array,
    A_wq: jax.Array,
    A_wo: jax.Array,
    B_x: jax.Array,
    B_w1: jax.Array,
    B_w2: jax.Array,
    B_w3: jax.Array,
    B_w4: jax.Array,
    c: jax.Array,
    w_mod: jax.Array,
):
    keys = A_k_cache.shape[2]
    assert A_x.shape == (1, 1, D) and A_k_cache.shape == (1, HKV, keys, DH)
    assert min(4096, max(256, keys // 4)) == WINDOW and keys % BLOCK == 0
    k, v = A_k_cache.reshape(-1, BLOCK, DH), A_v_cache.reshape(-1, BLOCK, DH)
    wm, wq, wo = w_mod.reshape(4, -1, 6 * D), A_wq.reshape(7, -1, HQ * DH), A_wo.T.reshape(7, -1, HQ * DH)
    w3, w4 = B_w3.reshape(2, -1, F), B_w4.T.reshape(7, -1, F)
    window = (HKV, WINDOW // BLOCK, BLOCK, DH)
    hbm = pl.BlockSpec(memory_space=pltpu.HBM)
    return pl.pallas_call(
        _kernel,
        out_shape=jax.ShapeDtypeStruct(A_x.shape, A_x.dtype),
        in_specs=[hbm] * 9,
        out_specs=hbm,
        scratch_shapes=[pltpu.VMEM(shape, BF16) for shape in (
            A_x.shape, c.shape, wm.shape, wq.shape, window, window, wo.shape, w3.shape, w4.shape)] + [
            pltpu.VMEM((HKV, ROWS, DH), F32),
            pltpu.VMEM((HKV, ROWS, WINDOW), F32),
            pltpu.VMEM((HKV, ROWS, DH), F32),
            pltpu.VMEM((ROWS, D), F32),
            pltpu.VMEM((6, ROWS, D), F32),
            pltpu.VMEM((D, LANES), F32),
            pltpu.VMEM(A_x.shape, BF16),
            pltpu.VMEM(A_x.shape, BF16),
            pltpu.SemaphoreType.DMA((S_END,)),
        ],
        compiler_params=pltpu.CompilerParams(
            vmem_limit_bytes=100 * 2**20,
            disable_semaphore_checks=True,
        ),
        name="adaln_decode",
    )(A_x, c, wm, wq, k, v, wo, w3, w4)
```
